```python
import os as _os
_os.environ.setdefault("JAX_PLATFORMS", "cpu")
import jax
import jax.numpy as jnp

def _softmax(x, axis=-1):
    return jax.nn.softmax(x, axis=axis)
def _gelu(x):
    return jax.nn.gelu(x, approximate=True)
def _silu(x):
    return jax.nn.silu(x)
def _sigmoid(x):
    return jax.nn.sigmoid(x)
def _layernorm(x, axis=-1, eps=1e-5):
    m = jnp.mean(x, axis=axis, keepdims=True)
    v = jnp.var(x, axis=axis, keepdims=True)
    return (x - m) / jnp.sqrt(v + eps)
def _scatter_add(tgt, idx, src, axis=0):
    return tgt.at[idx].add(src)
def _segment_sum(src, seg, n):
    return jax.ops.segment_sum(src, seg, n)
class _Rng:
    def __init__(self, key):
        self._k = key
    def _next(self):
        self._k, sub = jax.random.split(self._k)
        return sub
    def normal(self, shape):
        return jax.random.normal(self._next(), shape, dtype=jnp.bfloat16)
    def randint(self, lo, hi, shape):
        return jax.random.randint(self._next(), shape, lo, hi, dtype=jnp.int32)
    def uniform(self, shape, lo=0.0, hi=1.0):
        return jax.random.uniform(self._next(), shape, jnp.bfloat16, lo, hi)
    def permutation(self, n):
        return jax.random.permutation(self._next(), n)


kernel_name = 'sequential_preLN__softmax_full_mha__mixer_channel_mlp__prompt'

def setup_inputs():
    _rng = _Rng(jax.random.key(int.from_bytes(__import__("os").urandom(4), "little")))
    _w = (lambda a: (lambda t: t.astype(jnp.bfloat16) if jnp.issubdtype(t.dtype, jnp.floating) else t)(jnp.asarray(a)))
    def _A_setup():
        B, S, D = 1, 2048, 1024
        return {
            "x": _w((lambda *s: _rng.normal(s) * 0.05)(B, S, D)),
            "wqkv": _w((lambda *s: _rng.normal(s) * 0.05)(D, 3 * D)),
            "wo": _w((lambda *s: _rng.normal(s) * 0.05)(D, D)),
        }
    _A_in = _A_setup()

    def _B_setup():
        B, S, D, F = 1, 2048, 1024, 3584
        return {
            "x": _w((lambda *s: _rng.normal(s) * 0.05)(B, S, D)),
            "w1": _w((lambda *s: _rng.normal(s) * 0.8)(D, F) * (D ** -0.5)),
            "b1": _w((lambda *s: _rng.normal(s) * 0.8)(F)),
            "w2": _w((lambda *s: _rng.normal(s) * 0.8)(F, D) * (F ** -0.5)),
            "b2": _w((lambda *s: _rng.normal(s) * 0.05)(D)),
        }
    _B_in = _B_setup()

    return {
        "A_x": _A_in["x"],
        "A_wqkv": _A_in["wqkv"],
        "A_wo": _A_in["wo"],
        "B_x": _B_in["x"],
        "B_w1": _B_in["w1"],
        "B_b1": _B_in["b1"],
        "B_w2": _B_in["w2"],
        "B_b2": _B_in["b2"],
    }

def reference(A_x, A_wqkv, A_wo, B_x, B_w1, B_b1, B_w2, B_b2):
    def _A_ref(x, wqkv, wo):
        B, S, D = x.shape
        H = 32; Dh = D // H
        qkv = (lambda x, *d: x.transpose(*d))((x @ wqkv).reshape(B, S, 3, H, Dh), 2, 0, 3, 1, 4)
        q, k, v = qkv[0], qkv[1], qkv[2]
        scale = Dh ** -0.5
        scores = jnp.einsum("bhqd,bhkd->bhqk", q, k) * scale
        p = _softmax(scores, axis=-1)
        o = jnp.einsum("bhqk,bhkd->bhqd", p, v)
        return (lambda x, *d: x.transpose(*d))(o, 0, 2, 1, 3).reshape(B, S, D) @ wo

    def _B_ref(x, w1, b1, w2, b2):
        y = _layernorm(x, axis=-1)
        h = _gelu(jnp.einsum("bsd,df->bsf", y, w1) + b1)
        return jnp.einsum("bsf,fd->bsd", h, w2) + b2

    x = A_x
    h = x + _A_ref(_layernorm(x, axis=-1), A_wqkv, A_wo)
    h2 = h + _B_ref(_layernorm(h, axis=-1), B_w1, B_b1, B_w2, B_b2)
    return h2
```

```python
import functools

import jax
import jax.numpy as jnp
from jax import lax
import jax.experimental.pallas as pl
import jax.experimental.pallas.tpu as pltpu

BF = jnp.bfloat16
F32 = jnp.float32

H = 32
EPS = 1e-5
LOG2E = 1.4426950408889634

TM1 = 512
TN1 = 512
SB1 = 128
TQ = 512
CK = 128
NS = 4
TM3 = 512
FC = 512
SB3 = 128


def _layernorm(x):
    mu = jnp.mean(x, axis=-1, keepdims=True)
    xc = x - mu
    var = jnp.mean(xc * xc, axis=-1, keepdims=True)
    return xc * lax.rsqrt(var + EPS)


def _gelu_tanh(x):
    c = 0.7978845608028654
    return 0.5 * x * (1.0 + jnp.tanh(c * (x + 0.044715 * (x * x * x))))


def _kernel(x_hbm, wqkv_hbm, wo_hbm, w1_hbm, b1_hbm, w2_hbm, b2_hbm, out_hbm,
            x_s, wqkv_s, wo_s, w1_s, b1_s, w2_s, b2_s,
            xn_s, k_s, qt_s, vt_s, ot_s, s_buf, m_s, h_s, y_s, o_s,
            sem_x, sem_w, sem_p, sem_o, *, S, D, F):
    DH = D // H
    G = D // 128
    qscale = (DH ** -0.5) * LOG2E
    n1 = S // TM1
    nw = 3 * D // TN1
    npart = D // TN1
    w_order = ([npart + n for n in range(npart)] + list(range(npart))
               + [2 * npart + n for n in range(npart)])

    def x_copy(i):
        return pltpu.make_async_copy(x_hbm.at[0, pl.ds(i * TM1, TM1), :],
                                     x_s.at[pl.ds(i * TM1, TM1), :], sem_x.at[i])

    def w_copy(n):
        return pltpu.make_async_copy(wqkv_hbm.at[:, pl.ds(n * TN1, TN1)],
                                     wqkv_s.at[:, pl.ds(n * TN1, TN1)], sem_w.at[n])

    p_copies = [pltpu.make_async_copy(src, dst, sem_p.at[n]) for n, (src, dst) in enumerate(
        ((wo_hbm, wo_s), (w1_hbm, w1_s), (w2_hbm, w2_s), (b1_hbm, b1_s), (b2_hbm, b2_s)))]

    def o_copy(r):
        return pltpu.make_async_copy(o_s.at[pl.ds(r, SB3), :],
                                     out_hbm.at[0, pl.ds(r, SB3), :], sem_o)

    x_copy(0).start()
    for n in w_order:
        w_copy(n).start()
    for i in range(1, n1):
        x_copy(i).start()
    for c in p_copies:
        c.start()

    def qkv_body(i, carry):
        r0 = pl.multiple_of(i * TM1, TM1)
        x_copy(i).wait()

        def wait_w(n):
            @pl.when(i == 0)
            def _():
                w_copy(n).wait()

        def store_k(n, kk, rows):
            kb = kk.astype(BF)
            for g in range(TN1 // 128):
                k_s[n * (TN1 // 128) + g, rows, :] = kb[:, g * 128:(g + 1) * 128]

        wait_w(npart)
        for r in range(TM1 // SB1):
            rr = pl.multiple_of(r0 + r * SB1, SB1)
            xn = _layernorm(x_s[pl.ds(rr, SB1), :].astype(F32)).astype(BF)
            xn_s[r * SB1:(r + 1) * SB1, :] = xn
            kk = jnp.dot(xn, wqkv_s[:, D:D + TN1], preferred_element_type=F32)
            store_k(0, kk, pl.ds(rr, SB1))
        for n in range(1, npart):
            wait_w(npart + n)
            kk = jnp.dot(xn_s[...], wqkv_s[:, D + n * TN1:D + (n + 1) * TN1],
                         preferred_element_type=F32)
            store_k(n, kk, pl.ds(r0, TM1))
        for part, dst in ((0, qt_s), (2, vt_s)):
            for n in range(npart):
                wait_w(part * npart + n)
                c0 = part * D + n * TN1
                t = lax.dot_general(wqkv_s[:, c0:c0 + TN1], xn_s[...],
                                    (((0,), (1,)), ((), ())), preferred_element_type=F32)
                if part == 0:
                    t = t * qscale
                t = t.astype(BF)
                for hh in range(TN1 // DH):
                    dst[n * (TN1 // DH) + hh, :, pl.ds(r0, TM1)] = t[hh * DH:(hh + 1) * DH, :]
        return carry

    lax.fori_loop(0, n1, qkv_body, 0)

    nq = S // TQ
    nck = S // CK
    nb = nq * G

    def load_qm(h, j, qi):
        qh = qt_s[h, :, pl.ds(pl.multiple_of(qi * TQ, TQ), TQ)]
        parts = []
        if j > 0:
            parts.append(jnp.zeros((DH * j, TQ), BF))
        parts.append(qh)
        if j < NS - 1:
            parts.append(jnp.zeros((DH * (NS - 1 - j), TQ), BF))
        return jnp.concatenate(parts, axis=0)

    def qk_chunk(i, g, qm, c, mrun):
        s = jnp.dot(k_s[g, c * CK:(c + 1) * CK, :], qm, preferred_element_type=F32)
        s_buf[i, c * CK:(c + 1) * CK, :] = s
        cm = jnp.max(s.reshape(CK // 8, 8, TQ), axis=0)
        return cm if mrun is None else jnp.maximum(mrun, cm)

    def pv_chunk(i, h, c, m, lrun, acc):
        ps = [None] * (CK // 16)
        cl = None
        for r in reversed(range(CK // 16)):
            s = s_buf[i, c * CK + r * 16:c * CK + (r + 1) * 16, :]
            p = jnp.exp2(s - m)
            cl = p[8:16] if cl is None else cl + p[8:16]
            cl = cl + p[0:8]
            ps[r] = p
        lrun = cl if lrun is None else lrun + cl
        pb = jnp.concatenate(ps, axis=0).astype(BF)
        o = jnp.dot(vt_s[h, :, c * CK:(c + 1) * CK], pb, preferred_element_type=F32)
        return lrun, (o if acc is None else acc + o)

    def attn_body(u, do_pv, do_qk):
        if do_pv:
            qi, g = u // G, u % G
        if do_qk:
            qin, gn = (u + 1) // G, (u + 1) % G
        for j in range(NS):
            if do_pv:
                h = g * NS + j
                m = m_s[j]
            if do_qk:
                qm = load_qm(gn * NS + j, j, qin)
            lrun = acc = mrun = None
            for c in range(nck):
                if do_pv:
                    lrun, acc = pv_chunk(j, h, c, m, lrun, acc)
                if do_qk:
                    mrun = qk_chunk(j, gn, qm, c, mrun)
            if do_pv:
                l = jnp.sum(lrun, axis=0, keepdims=True)
                ot_s[pl.ds(pl.multiple_of(h * DH, DH), DH),
                     pl.ds(pl.multiple_of(qi * TQ, TQ), TQ)] = (acc / l).astype(BF)
            if do_qk:
                m_s[j] = jnp.max(mrun, axis=0, keepdims=True)

    attn_body(-1, False, True)

    def attn_loop(u, carry):
        attn_body(u, True, True)
        return carry

    lax.fori_loop(0, nb - 1, attn_loop, 0)
    attn_body(nb - 1, True, False)

    for c in p_copies:
        c.wait()
    n3 = S // TM3
    nf = F // FC
    nsb = TM3 // SB3

    def mlp_body(i, carry):
        r0 = pl.multiple_of(i * TM3, TM3)
        for r in range(nsb):
            rr = pl.multiple_of(r0 + r * SB3, SB3)
            at = lax.dot_general(ot_s[:, pl.ds(rr, SB3)], wo_s[...],
                                 (((0,), (0,)), ((), ())), preferred_element_type=F32)
            h = x_s[pl.ds(rr, SB3), :].astype(F32) + at
            h_s[r * SB3:(r + 1) * SB3, :] = h
            y_s[r * SB3:(r + 1) * SB3, :] = _layernorm(_layernorm(h)).astype(BF)

        def up(c, sub):
            w = w1_s[:, c * FC:(c + 1) * FC]
            b = b1_s[:, c * FC:(c + 1) * FC].astype(F32)
            if sub:
                parts = [_gelu_tanh(jnp.dot(y_s[r * SB3:(r + 1) * SB3, :], w,
                                            preferred_element_type=F32) + b)
                         for r in range(nsb)]
                return jnp.concatenate(parts, axis=0).astype(BF)
            return _gelu_tanh(jnp.dot(y_s[...], w, preferred_element_type=F32) + b).astype(BF)

        acc = None
        g_next = up(0, True)
        for c in range(nf):
            g_cur = g_next
            if c + 1 < nf:
                g_next = up(c + 1, False)
            w2 = w2_s[c * FC:(c + 1) * FC, :]
            if c + 1 < nf:
                p = jnp.dot(g_cur, w2, preferred_element_type=F32)
                acc = p if acc is None else acc + p
            else:
                for r in range(nsb):
                    rr = pl.multiple_of(r0 + r * SB3, SB3)
                    p = jnp.dot(g_cur[r * SB3:(r + 1) * SB3], w2, preferred_element_type=F32)
                    res = (acc[r * SB3:(r + 1) * SB3] + p + b2_s[...].astype(F32)
                           + h_s[r * SB3:(r + 1) * SB3, :])
                    o_s[pl.ds(rr, SB3), :] = res.astype(BF)
                    o_copy(rr).start()
        return carry

    lax.fori_loop(0, n3, mlp_body, 0)
    for r in range(S // SB3):
        o_copy(r * SB3).wait()


@jax.jit
def pallas_sequential_preLN__softmax_full_mha__mixer_channel_mlp__prompt_kernel(
    A_x: jax.Array,
    A_wqkv: jax.Array,
    A_wo: jax.Array,
    B_x: jax.Array,
    B_w1: jax.Array,
    B_b1: jax.Array,
    B_w2: jax.Array,
    B_b2: jax.Array,
):
    B, S, D = A_x.shape
    F = B_w1.shape[1]
    assert B == 1 and D % 128 == 0 and (D // H) * NS == 128
    DH = D // H
    G = D // 128
    any_spec = pl.BlockSpec(memory_space=pl.ANY)
    return pl.pallas_call(
        functools.partial(_kernel, S=S, D=D, F=F),
        out_shape=jax.ShapeDtypeStruct((B, S, D), A_x.dtype),
        in_specs=[any_spec] * 7,
        out_specs=any_spec,
        scratch_shapes=[
            pltpu.VMEM((S, D), BF),
            pltpu.VMEM((D, 3 * D), BF),
            pltpu.VMEM((D, D), BF),
            pltpu.VMEM((D, F), BF),
            pltpu.VMEM((1, F), BF),
            pltpu.VMEM((F, D), BF),
            pltpu.VMEM((1, D), BF),
            pltpu.VMEM((TM1, D), BF),
            pltpu.VMEM((G, S, 128), BF),
            pltpu.VMEM((H, DH, S), BF),
            pltpu.VMEM((H, DH, S), BF),
            pltpu.VMEM((D, S), BF),
            pltpu.VMEM((NS, S, TQ), F32),
            pltpu.VMEM((NS, 1, TQ), F32),
            pltpu.VMEM((TM3, D), F32),
            pltpu.VMEM((TM3, D), BF),
            pltpu.VMEM((S, D), BF),
            pltpu.SemaphoreType.DMA((S // TM1,)),
            pltpu.SemaphoreType.DMA((3 * D // TN1,)),
            pltpu.SemaphoreType.DMA((5,)),
            pltpu.SemaphoreType.DMA(()),
        ],
        compiler_params=pltpu.CompilerParams(vmem_limit_bytes=110 * 1024 * 1024),
    )(A_x, A_wqkv, A_wo, B_w1, B_b1.reshape(1, F), B_w2, B_b2.reshape(1, D))
```

```python
import functools

import jax
import jax.numpy as jnp
from jax import lax
import jax.experimental.pallas as pl
import jax.experimental.pallas.tpu as pltpu

BF = jnp.bfloat16
F32 = jnp.float32

H = 32
EPS = 1e-5
LOG2E = 1.4426950408889634

TM1 = 512
TN1 = 512
SB1 = 128
LNB = 32
TQ = 512
CK = 128
HPG = 4
NS = 8
OPM = 128
OPN = 256
TM3 = 256
FC = 512
SB3 = 128


def _layernorm(x):
    mu = jnp.mean(x, axis=-1, keepdims=True)
    xc = x - mu
    var = jnp.mean(xc * xc, axis=-1, keepdims=True)
    return xc * lax.rsqrt(var + EPS)


def _gelu_tanh(x):
    c = 0.7978845608028654
    return 0.5 * x * (1.0 + jnp.tanh(c * (x + 0.044715 * (x * x * x))))


def _tie(v, y):
    if y is None:
        return v
    w = v.shape[1]
    t = jnp.max(y.reshape(y.shape[0] // 8, 8, y.shape[1]), axis=0)
    tw = t[:, :w]
    for k in range(1, y.shape[1] // w):
        tw = jnp.maximum(tw, t[:, k * w:(k + 1) * w])
    return jnp.where(tw > jnp.inf, tw, v)


def _interleave(main, extra):
    n, k = len(main), len(extra)
    done = 0
    for idx, fn in enumerate(main):
        fn()
        want = ((idx + 1) * k) // n
        while done < want:
            extra[done]()
            done += 1


def _kernel(x_hbm, wqkv_hbm, wo_hbm, w1_hbm, b1_hbm, w2_hbm, b2_hbm, out_hbm,
            s_buf, k_s, qt_s, vt_s, o_s, h_s, y_s, yn_s, x_s, xn_s, wqkv_s, wo_s, w1_s, w2_s,
            ot_t, m_s, b1_s, b2_s,
            sem_x, sem_w, sem_p, sem_o, *, S, D, F):
    DH = D // H
    G = D // 128
    qscale = (DH ** -0.5) * LOG2E
    n1 = S // TM1
    npart = D // TN1
    w_order = ([npart + n for n in range(npart)] + list(range(npart))
               + [2 * npart + n for n in range(npart)])

    nsb1 = TM1 // SB1
    x_rows = ([(r * SB1, SB1) for r in range(nsb1)]
              + [(i * TM1, TM1) for i in range(1, n1)])
    c_first = w_order[0] * TN1
    w_cols = ([(c_first, TN1 // 2), (c_first + TN1 // 2, TN1 // 2)]
              + [(n * TN1, TN1) for n in w_order[1:]])

    def x_copy(i):
        r0, nr = x_rows[i]
        return pltpu.make_async_copy(x_hbm.at[0, pl.ds(r0, nr), :],
                                     x_s.at[pl.ds(r0, nr), :], sem_x.at[i])

    def w_copy(n):
        c0, nc = w_cols[n]
        return pltpu.make_async_copy(wqkv_hbm.at[:, pl.ds(c0, nc)],
                                     wqkv_s.at[:, pl.ds(c0, nc)], sem_w.at[n])

    p_copies = [pltpu.make_async_copy(src, dst, sem_p.at[n]) for n, (src, dst) in enumerate(
        ((wo_hbm, wo_s), (w1_hbm, w1_s), (w2_hbm, w2_s), (b1_hbm, b1_s), (b2_hbm, b2_s)))]

    def o_copy(r):
        return pltpu.make_async_copy(x_s.at[pl.ds(r, SB3), :],
                                     out_hbm.at[0, pl.ds(r, SB3), :], sem_o)

    def ln1(i, r):
        for rr in range(r * SB1, (r + 1) * SB1, LNB):
            xb = x_s[i * TM1 + rr:i * TM1 + rr + LNB, :].astype(F32)
            xn_s[i % 2, rr:rr + LNB, :] = _layernorm(xb).astype(BF)

    def proj(i, n, r=None, half=None):
        c0, nc = n * TN1, TN1
        if half is not None:
            nc = TN1 // 2
            c0 += half * nc
        part = c0 // D
        lo, hi = (0, TM1) if r is None else (r * SB1, (r + 1) * SB1)
        rows = slice(i * TM1 + lo, i * TM1 + hi)
        xn = xn_s[i % 2, lo:hi, :]
        if part == 1:
            kb = jnp.dot(xn, wqkv_s[:, c0:c0 + nc], preferred_element_type=F32).astype(BF)
            for g in range(nc // 128):
                k_s[(c0 - D) // 128 + g, rows, :] = kb[:, g * 128:(g + 1) * 128]
        else:
            t = lax.dot_general(wqkv_s[:, c0:c0 + nc], xn,
                                (((0,), (1,)), ((), ())), preferred_element_type=F32)
            if part == 0:
                t = t * qscale
            t = t.astype(BF)
            dst = qt_s if part == 0 else vt_s
            for hh in range(nc // DH):
                dst[(c0 - part * D) // DH + hh, :, rows] = t[hh * DH:(hh + 1) * DH, :]

    def head_work(i):
        def blk(r):
            def fn():
                ln1(i, r)
                proj(i, w_order[0], r)
            return fn
        return [blk(r) for r in range(nsb1)]

    def tail_work(i, first=1):
        return [functools.partial(proj, i, n) for n in w_order[first:]]

    for r in range(nsb1):
        x_copy(r).start()
    for r in range(nsb1):
        x_copy(r).wait()
        if r == 0:
            for n in range(len(w_cols)):
                w_copy(n).start()
        ln1(0, r)
    w_copy(0).wait()
    for r in range(nsb1, len(x_rows)):
        x_copy(r).start()
    proj(0, w_order[0], half=0)
    w_copy(1).wait()
    for c in p_copies:
        c.start()
    proj(0, w_order[0], half=1)
    w_copy(2).wait()
    proj(0, w_order[1])
    w_copy(3).wait()
    w_copy(4).wait()
    proj(0, w_order[2])
    proj(0, w_order[3])
    for n in range(5, len(w_cols)):
        w_copy(n).wait()
    x_copy(nsb1).wait()
    _interleave(tail_work(0, 4), head_work(1))
    for r in range(nsb1 + 1, len(x_rows)):
        x_copy(r).wait()
    for i in range(1, n1):
        _interleave(tail_work(i), head_work(i + 1) if i + 1 < n1 else [])

    nq = S // TQ
    nck = S // CK
    gpb = NS // HPG
    gb = G // gpb
    nb = nq * gb

    def load_qm(h, j, qi):
        qh = qt_s[h, :, pl.ds(pl.multiple_of(qi * TQ, TQ), TQ)]
        parts = []
        if j > 0:
            parts.append(jnp.zeros((DH * j, TQ), BF))
        parts.append(qh)
        if j < HPG - 1:
            parts.append(jnp.zeros((DH * (HPG - 1 - j), TQ), BF))
        return jnp.concatenate(parts, axis=0)

    def qk_chunk(i, g, qm, c, mrun):
        s = jnp.dot(k_s[g, c * CK:(c + 1) * CK, :], qm, preferred_element_type=F32)
        s_buf[i, c * CK:(c + 1) * CK, :] = s
        cm = jnp.max(s.reshape(CK // 8, 8, TQ), axis=0)
        return cm if mrun is None else jnp.maximum(mrun, cm)

    def p_chunk(i, c, m, lrun):
        ps = [None] * (CK // 16)
        cl = None
        for r in reversed(range(CK // 16)):
            s = s_buf[i, c * CK + r * 16:c * CK + (r + 1) * 16, :]
            p = jnp.exp2(s - m)
            cl = p[8:16] if cl is None else cl + p[8:16]
            cl = cl + p[0:8]
            ps[r] = p
        lrun = cl if lrun is None else lrun + cl
        return lrun, jnp.concatenate(ps, axis=0).astype(BF)

    def pv_chunk(h, c, pb, acc):
        o = jnp.dot(vt_s[h, :, c * CK:(c + 1) * CK], pb, preferred_element_type=F32)
        return o if acc is None else o + acc

    def flush_o(u):
        qi, g0 = u // gb, (u % gb) * gpb
        for gg in range(gpb):
            o_s[g0 + gg, pl.ds(pl.multiple_of(qi * TQ, TQ), TQ), :] = (
                ot_t[gg * 128:(gg + 1) * 128, :].T.astype(BF))

    def attn_work(u, do_pv, do_qk):
        if do_pv:
            qi, g0 = u // gb, (u % gb) * gpb
        if do_qk:
            qin, gn0 = (u + 1) // gb, ((u + 1) % gb) * gpb
        work = []
        for i in range(NS):
            j = i % HPG
            st = {}

            def step(c, i=i, j=j, st=st):
                if do_pv:
                    h = (g0 + i // HPG) * HPG + j
                    if c == 0:
                        st['m'] = m_s[i]
                        st['l'] = st['acc'] = None
                    st['l'], pb = p_chunk(i, c, st['m'], st['l'])
                if do_qk:
                    gn = gn0 + i // HPG
                    if c == 0:
                        st['qm'] = load_qm(gn * HPG + j, j, qin)
                        st['mrun'] = None
                    st['mrun'] = qk_chunk(i, gn, st['qm'], c, st['mrun'])
                if do_pv:
                    st['acc'] = pv_chunk(h, c, pb, st['acc'])
                if c == nck - 1:
                    if do_pv:
                        l = jnp.sum(st['l'], axis=0, keepdims=True)
                        ot_t[i * DH:(i + 1) * DH, :] = st['acc'] / l
                    if do_qk:
                        m_s[i] = jnp.max(st['mrun'], axis=0, keepdims=True)
            work += [functools.partial(step, c) for c in range(nck)]
        return work

    ot_t[...] = jnp.zeros(ot_t.shape, F32)
    h_s[S:S + TM3, :] = jnp.zeros((TM3, D), F32)
    for fn in attn_work(-1, False, True):
        fn()

    def attn_loop(u, carry):
        flush_o(jnp.maximum(u - 1, 0))
        for fn in attn_work(u, True, True):
            fn()
        return carry

    lax.fori_loop(0, nb - 1, attn_loop, 0)

    def op_work(r0, nrows, ncols):
        rows = slice(r0, r0 + nrows)

        def piece(n):
            def fn(dep=None):
                o = jnp.concatenate([o_s[g, rows, :] for g in range(G)], axis=1)
                cols = slice(n * ncols, (n + 1) * ncols)
                at = jnp.dot(o, wo_s[:, cols], preferred_element_type=F32)
                xr = x_s[rows, cols].astype(F32)
                if dep is not None:
                    xr = jnp.concatenate([_tie(xr[:8], dep), xr[8:]], axis=0)
                h_s[rows, cols] = xr + at
                return at
            return fn
        return [piece(n) for n in range(D // ncols)]

    def op_small_work(r0):
        rows = slice(r0, r0 + CK)

        def piece(n, g):
            def fn():
                cols = slice(n * TQ, (n + 1) * TQ)
                at = jnp.dot(o_s[g, rows, :], wo_s[g * 128:(g + 1) * 128, cols],
                             preferred_element_type=F32)
                prev = x_s[rows, cols].astype(F32) if g == 0 else h_s[rows, cols]
                h_s[rows, cols] = prev + at
            return fn
        return [piece(n, g) for n in range(D // TQ) for g in range(G)]

    def ln2(dst, r0, b, dep=None):
        hb = h_s[pl.ds(pl.multiple_of(r0 + b * LNB, LNB), LNB), :]
        if dep is not None:
            w = dep.shape[1]
            head = [_tie(hb[k * 8:(k + 1) * 8, :w], dep) for k in range(LNB // 8)]
            hb = jnp.concatenate([jnp.concatenate(head, axis=0), hb[:, w:]], axis=1)
        y = _layernorm(_layernorm(hb))
        dst[b * LNB:(b + 1) * LNB, :] = y.astype(BF)
        return y

    for c in p_copies:
        c.wait()
    flush_o(nb - 2)
    epi = attn_work(nb - 1, True, False)
    fused_rows = (len(epi) // (G * (D // TQ))) * CK
    extra = []
    for r0 in range(0, fused_rows, CK):
        extra += op_small_work(r0)
    _interleave(epi, extra)
    flush_o(nb - 1)
    rest = []
    for r0 in range(fused_rows, S, OPM):
        rest += op_work(r0, OPM, OPN)
    nln = TM3 // LNB
    step = len(rest) // nln
    gate = None
    for k, fn in enumerate(rest):
        at = fn(ln2(yn_s, 0, k // step, gate) if k % step == step - 1 else None)
        if k % step == 0:
            gate = at[:8]

    n3 = S // TM3
    nf = F // FC
    nsb = TM3 // SB3

    def mlp_body(i, carry):
        r0 = pl.multiple_of(i * TM3, TM3)
        y_s[...] = yn_s[...]

        blocks = list(range(nln))

        def next_ln():
            return ln2(yn_s, r0 + TM3, blocks.pop(0)) if blocks else None

        def up(c, dep):
            b = b1_s[pl.ds(c * FC, FC)].astype(F32).reshape(1, FC)
            b = _tie(jnp.broadcast_to(b, (8, FC)), dep)
            a = jnp.dot(y_s[...], w1_s[:, c * FC:(c + 1) * FC],
                        preferred_element_type=F32)
            a = (a.reshape(TM3 // 8, 8, FC) + b[None]).reshape(TM3, FC)
            return _gelu_tanh(a).astype(BF)

        acc = None
        g_next = up(0, None)
        for c in range(nf):
            g_cur = g_next
            if c + 1 < nf:
                g_next = up(c + 1, next_ln())
            w2 = w2_s[c * FC:(c + 1) * FC, :]
            if c + 1 < nf:
                p = jnp.dot(g_cur, w2, preferred_element_type=F32)
                acc = p if acc is None else p + acc
            else:
                b2 = jnp.broadcast_to(b2_s[...].astype(F32).reshape(1, D), (8, D))
                for r in range(nsb):
                    rr = pl.multiple_of(r0 + r * SB3, SB3)
                    b2r = _tie(b2, next_ln())
                    p = jnp.dot(g_cur[r * SB3:(r + 1) * SB3], w2, preferred_element_type=F32)
                    res = p + acc[r * SB3:(r + 1) * SB3] + h_s[pl.ds(rr, SB3), :]
                    res = (res.reshape(SB3 // 8, 8, D) + b2r[None]).reshape(SB3, D)
                    x_s[pl.ds(rr, SB3), :] = res.astype(BF)
                    o_copy(rr).start()
        while blocks:
            next_ln()
        return carry

    lax.fori_loop(0, n3, mlp_body, 0)
    for r in range(S // SB3):
        o_copy(r * SB3).wait()


@jax.jit
def pallas_sequential_preLN__softmax_full_mha__mixer_channel_mlp__prompt_kernel(
    A_x: jax.Array,
    A_wqkv: jax.Array,
    A_wo: jax.Array,
    B_x: jax.Array,
    B_w1: jax.Array,
    B_b1: jax.Array,
    B_w2: jax.Array,
    B_b2: jax.Array,
):
    B, S, D = A_x.shape
    F = B_w1.shape[1]
    assert B == 1 and D % 128 == 0 and (D // H) * HPG == 128
    DH = D // H
    G = D // 128
    any_spec = pl.BlockSpec(memory_space=pl.ANY)
    return pl.pallas_call(
        functools.partial(_kernel, S=S, D=D, F=F),
        out_shape=jax.ShapeDtypeStruct((B, S, D), A_x.dtype),
        in_specs=[any_spec] * 7,
        out_specs=any_spec,
        scratch_shapes=[
            pltpu.VMEM((NS, S, TQ), F32),
            pltpu.VMEM((G, S, 128), BF),
            pltpu.VMEM((H, DH, S), BF),
            pltpu.VMEM((H, DH, S), BF),
            pltpu.VMEM((G, S, 128), BF),
            pltpu.VMEM((S + TM3, D), F32),
            pltpu.VMEM((TM3, D), BF),
            pltpu.VMEM((TM3, D), BF),
            pltpu.VMEM((S, D), BF),
            pltpu.VMEM((2, TM1, D), BF),
            pltpu.VMEM((D, 3 * D), BF),
            pltpu.VMEM((D, D), BF),
            pltpu.VMEM((D, F), BF),
            pltpu.VMEM((F, D), BF),
            pltpu.VMEM((NS * DH, TQ), F32),
            pltpu.VMEM((NS, 1, TQ), F32),
            pltpu.VMEM((F,), BF),
            pltpu.VMEM((D,), BF),
            pltpu.SemaphoreType.DMA((TM1 // SB1 + S // TM1 - 1,)),
            pltpu.SemaphoreType.DMA((3 * D // TN1 + 1,)),
            pltpu.SemaphoreType.DMA((5,)),
            pltpu.SemaphoreType.DMA(()),
        ],
        compiler_params=pltpu.CompilerParams(vmem_limit_bytes=120 * 1024 * 1024),
    )(A_x, A_wqkv, A_wo, B_w1, B_b1, B_w2, B_b2)
```

```python
import functools

import jax
import jax.numpy as jnp
from jax import lax
import jax.experimental.pallas as pl
import jax.experimental.pallas.tpu as pltpu

BF = jnp.bfloat16
F32 = jnp.float32

H = 32
EPS = 1e-5
LOG2E = 1.4426950408889634

TM1 = 512
TN1 = 512
SB1 = 128
LNB = 32
TQ = 512
CK = 128
HPG = 4
NS = 8
OPM = 128
OPN = 256
TM3 = 256
FC = 512
SB3 = 128


def _layernorm(x):
    mu = jnp.mean(x, axis=-1, keepdims=True)
    xc = x - mu
    var = jnp.mean(xc * xc, axis=-1, keepdims=True)
    return xc * lax.rsqrt(var + EPS)


def _gelu_tanh(x):
    c = 0.7978845608028654
    return 0.5 * x * (1.0 + jnp.tanh(c * (x + 0.044715 * (x * x * x))))


def _tie(v, y):
    if y is None:
        return v
    w = v.shape[1]
    t = jnp.max(y.reshape(y.shape[0] // 8, 8, y.shape[1]), axis=0)
    tw = t[:, :w]
    for k in range(1, y.shape[1] // w):
        tw = jnp.maximum(tw, t[:, k * w:(k + 1) * w])
    return jnp.where(tw > jnp.inf, tw, v)


def _interleave(main, extra):
    n, k = len(main), len(extra)
    done = 0
    for idx, fn in enumerate(main):
        fn()
        want = ((idx + 1) * k) // n
        while done < want:
            extra[done]()
            done += 1


def _kernel(x_hbm, wqkv_hbm, wo_hbm, w1_hbm, b1_hbm, w2_hbm, b2_hbm, out_hbm,
            s_buf, k_s, qt_s, vt_s, o_s, h_s, y_s, yn_s, x_s, xn_s, wqkv_s, wo_s, w1_s, w2_s,
            ot_t, m_s, b1_s, b2_s,
            sem_x, sem_w, sem_p, sem_o, *, S, D, F):
    DH = D // H
    G = D // 128
    qscale = (DH ** -0.5) * LOG2E
    n1 = S // TM1
    npart = D // TN1
    w_order = ([npart + n for n in range(npart)] + list(range(npart))
               + [2 * npart + n for n in range(npart)])

    nsb1 = TM1 // SB1
    x_rows = ([(r * SB1, SB1) for r in range(nsb1)]
              + [(i * TM1, TM1) for i in range(1, n1)])
    c_first = w_order[0] * TN1
    wsb = TN1 // 2
    dma_order = [w_order[2], w_order[1]] + w_order[3:]
    w_cols = ([(c_first + b * wsb, wsb) for b in range(2)]
              + [(n * TN1, TN1) for n in dma_order])

    def x_copy(i):
        r0, nr = x_rows[i]
        return pltpu.make_async_copy(x_hbm.at[0, pl.ds(r0, nr), :],
                                     x_s.at[pl.ds(r0, nr), :], sem_x.at[i])

    def w_copy(n):
        c0, nc = w_cols[n]
        return pltpu.make_async_copy(wqkv_hbm.at[:, pl.ds(c0, nc)],
                                     wqkv_s.at[:, pl.ds(c0, nc)], sem_w.at[n])

    p_copies = [pltpu.make_async_copy(src, dst, sem_p.at[n]) for n, (src, dst) in enumerate(
        ((wo_hbm, wo_s), (w1_hbm, w1_s), (w2_hbm, w2_s), (b1_hbm, b1_s), (b2_hbm, b2_s)))]

    def o_copy(r):
        return pltpu.make_async_copy(x_s.at[pl.ds(r, SB3), :],
                                     out_hbm.at[0, pl.ds(r, SB3), :], sem_o)

    def ln1(i, r):
        for rr in range(r * SB1, (r + 1) * SB1, LNB):
            xb = x_s[i * TM1 + rr:i * TM1 + rr + LNB, :].astype(F32)
            xn_s[i % 2, rr:rr + LNB, :] = _layernorm(xb).astype(BF)

    def proj(i, n, r=None, cols=None):
        c0, nc = n * TN1, TN1
        if cols is not None:
            c0, nc = c0 + cols[0] * wsb, (cols[1] - cols[0]) * wsb
        part = c0 // D
        lo, hi = (0, TM1) if r is None else (r[0] * SB1, r[1] * SB1)
        rows = slice(i * TM1 + lo, i * TM1 + hi)
        xn = xn_s[i % 2, lo:hi, :]
        if part == 1:
            kb = jnp.dot(xn, wqkv_s[:, c0:c0 + nc], preferred_element_type=F32).astype(BF)
            for g in range(nc // 128):
                k_s[(c0 - D) // 128 + g, rows, :] = kb[:, g * 128:(g + 1) * 128]
        else:
            t = lax.dot_general(wqkv_s[:, c0:c0 + nc], xn,
                                (((0,), (1,)), ((), ())), preferred_element_type=F32)
            if part == 0:
                t = t * qscale
            t = t.astype(BF)
            dst = qt_s if part == 0 else vt_s
            for hh in range(nc // DH):
                dst[(c0 - part * D) // DH + hh, :, rows] = t[hh * DH:(hh + 1) * DH, :]

    def head_work(i):
        def blk(r):
            def fn():
                ln1(i, r)
                proj(i, w_order[0], (r, r + 1))
            return fn
        return [blk(r) for r in range(nsb1)]

    def tail_work(i, first=1):
        return [functools.partial(proj, i, n) for n in w_order[first:]]

    hb = nsb1 // 2
    for r in range(hb):
        x_copy(r).start()
    for r in range(hb):
        x_copy(r).wait()
        if r == 0:
            w_copy(0).start()
        if r == hb - 1:
            for rr in range(hb, nsb1):
                x_copy(rr).start()
        ln1(0, r)
    w_copy(0).wait()
    for n in range(1, len(w_cols)):
        w_copy(n).start()
    proj(0, w_order[0], (0, hb), (0, 1))
    for r in range(hb, nsb1):
        x_copy(r).wait()
    for r in range(nsb1, len(x_rows)):
        x_copy(r).start()
    for r in range(hb, nsb1):
        ln1(0, r)
        proj(0, w_order[0], (r, r + 1), (0, 1))
    w_copy(1).wait()
    for c in p_copies:
        c.start()
    proj(0, w_order[0], None, (1, 2))
    w_copy(2).wait()
    proj(0, w_order[2])
    w_copy(3).wait()
    w_copy(4).wait()
    proj(0, w_order[1], (0, hb))
    proj(0, w_order[3])
    for n in range(5, len(w_cols)):
        w_copy(n).wait()
    x_copy(nsb1).wait()
    proj(0, w_order[1], (hb, nsb1))
    _interleave(tail_work(0, 4), head_work(1))
    for r in range(nsb1 + 1, len(x_rows)):
        x_copy(r).wait()
    for i in range(1, n1):
        _interleave(tail_work(i), head_work(i + 1) if i + 1 < n1 else [])

    nq = S // TQ
    nck = S // CK
    gpb = NS // HPG
    gb = G // gpb
    nb = nq * gb

    def load_qm(h, j, qi):
        qh = qt_s[h, :, pl.ds(pl.multiple_of(qi * TQ, TQ), TQ)]
        parts = []
        if j > 0:
            parts.append(jnp.zeros((DH * j, TQ), BF))
        parts.append(qh)
        if j < HPG - 1:
            parts.append(jnp.zeros((DH * (HPG - 1 - j), TQ), BF))
        return jnp.concatenate(parts, axis=0)

    def qk_chunk(i, g, qm, c, mrun):
        s = jnp.dot(k_s[g, c * CK:(c + 1) * CK, :], qm, preferred_element_type=F32)
        s_buf[i, c * CK:(c + 1) * CK, :] = s
        cm = jnp.max(s.reshape(CK // 8, 8, TQ), axis=0)
        return cm if mrun is None else jnp.maximum(mrun, cm)

    def p_chunk(i, c, m, lrun):
        ps = [None] * (CK // 16)
        cl = None
        for r in reversed(range(CK // 16)):
            s = s_buf[i, c * CK + r * 16:c * CK + (r + 1) * 16, :]
            p = jnp.exp2(s - m)
            cl = p[8:16] if cl is None else cl + p[8:16]
            cl = cl + p[0:8]
            ps[r] = p
        lrun = cl if lrun is None else lrun + cl
        return lrun, jnp.concatenate(ps, axis=0).astype(BF)

    def pv_chunk(h, c, pb, acc):
        o = jnp.dot(vt_s[h, :, c * CK:(c + 1) * CK], pb, preferred_element_type=F32)
        return o if acc is None else o + acc

    def flush_o(u):
        qi, g0 = u // gb, (u % gb) * gpb
        for gg in range(gpb):
            o_s[g0 + gg, pl.ds(pl.multiple_of(qi * TQ, TQ), TQ), :] = (
                ot_t[gg * 128:(gg + 1) * 128, :].T.astype(BF))

    def attn_work(u, do_pv, do_qk):
        if do_pv:
            qi, g0 = u // gb, (u % gb) * gpb
        if do_qk:
            qin, gn0 = (u + 1) // gb, ((u + 1) % gb) * gpb
        work = []
        for i in range(NS):
            j = i % HPG
            st = {}

            def step(c, i=i, j=j, st=st):
                if do_pv:
                    h = (g0 + i // HPG) * HPG + j
                    if c == 0:
                        st['m'] = m_s[i]
                        st['l'] = st['acc'] = None
                    st['l'], pb = p_chunk(i, c, st['m'], st['l'])
                if do_qk:
                    gn = gn0 + i // HPG
                    if c == 0:
                        st['qm'] = load_qm(gn * HPG + j, j, qin)
                        st['mrun'] = None
                    st['mrun'] = qk_chunk(i, gn, st['qm'], c, st['mrun'])
                if do_pv:
                    st['acc'] = pv_chunk(h, c, pb, st['acc'])
                if c == nck - 1:
                    if do_pv:
                        l = jnp.sum(st['l'], axis=0, keepdims=True)
                        ot_t[i * DH:(i + 1) * DH, :] = st['acc'] / l
                    if do_qk:
                        m_s[i] = jnp.max(st['mrun'], axis=0, keepdims=True)
            work += [functools.partial(step, c) for c in range(nck)]
        return work

    ot_t[...] = jnp.zeros(ot_t.shape, F32)
    for fn in attn_work(-1, False, True):
        fn()

    def attn_loop(u, carry):
        flush_o(jnp.maximum(u - 1, 0))
        for fn in attn_work(u, True, True):
            fn()
        return carry

    lax.fori_loop(0, nb - 1, attn_loop, 0)

    def op_work(r0, nrows, ncols):
        rows = slice(r0, r0 + nrows)

        def piece(n):
            def fn(dep=None):
                o = jnp.concatenate([o_s[g, rows, :] for g in range(G)], axis=1)
                cols = slice(n * ncols, (n + 1) * ncols)
                at = jnp.dot(o, wo_s[:, cols], preferred_element_type=F32)
                xr = x_s[rows, cols].astype(F32)
                if dep is not None:
                    xr = jnp.concatenate([_tie(xr[:8], dep), xr[8:]], axis=0)
                h_s[rows, cols] = xr + at
                return at
            return fn
        return [piece(n) for n in range(D // ncols)]

    def op_small_work(r0):
        rows = slice(r0, r0 + CK)

        def piece(n, g):
            def fn():
                cols = slice(n * TQ, (n + 1) * TQ)
                at = jnp.dot(o_s[g, rows, :], wo_s[g * 128:(g + 1) * 128, cols],
                             preferred_element_type=F32)
                prev = x_s[rows, cols].astype(F32) if g == 0 else h_s[rows, cols]
                h_s[rows, cols] = prev + at
            return fn
        return [piece(n, g) for n in range(D // TQ) for g in range(G)]

    def ln2(dst, r0, b, dep=None):
        hb = h_s[pl.ds(pl.multiple_of(r0 + b * LNB, LNB), LNB), :]
        if dep is not None:
            w = dep.shape[1]
            head = [_tie(hb[k * 8:(k + 1) * 8, :w], dep) for k in range(LNB // 8)]
            hb = jnp.concatenate([jnp.concatenate(head, axis=0), hb[:, w:]], axis=1)
        y = _layernorm(_layernorm(hb))
        dst[b * LNB:(b + 1) * LNB, :] = y.astype(BF)
        return y

    for c in p_copies:
        c.wait()
    flush_o(nb - 2)
    epi = attn_work(nb - 1, True, False)
    fused_rows = (len(epi) // (G * (D // TQ))) * CK
    extra = []
    for r0 in range(0, fused_rows, CK):
        extra += op_small_work(r0)
    _interleave(extra, epi)
    flush_o(nb - 1)
    rest = []
    for r0 in range(fused_rows, S, OPM):
        rest += op_work(r0, OPM, OPN)
    nln = TM3 // LNB
    step = len(rest) // nln
    gate = None
    for k, fn in enumerate(rest):
        at = fn(ln2(yn_s, 0, k // step, gate) if k % step == step - 1 else None)
        if k % step == 0:
            gate = at[:8]

    n3 = S // TM3
    nf = F // FC
    nsb = TM3 // SB3

    def mlp_body(i, carry):
        r0 = pl.multiple_of(i * TM3, TM3)
        rn = jnp.minimum(i + 1, n3 - 1) * TM3
        y_s[...] = yn_s[...]

        blocks = list(range(nln))

        def next_ln():
            return ln2(yn_s, rn, blocks.pop(0)) if blocks else None

        def up(c, dep):
            b = b1_s[pl.ds(c * FC, FC)].astype(F32).reshape(1, FC)
            b = _tie(jnp.broadcast_to(b, (8, FC)), dep)
            a = jnp.dot(y_s[...], w1_s[:, c * FC:(c + 1) * FC],
                        preferred_element_type=F32)
            a = (a.reshape(TM3 // 8, 8, FC) + b[None]).reshape(TM3, FC)
            return _gelu_tanh(a).astype(BF)

        acc = None
        g_next = up(0, None)
        for c in range(nf):
            g_cur = g_next
            if c + 1 < nf:
                g_next = up(c + 1, next_ln())
            w2 = w2_s[c * FC:(c + 1) * FC, :]
            if c + 1 < nf:
                p = jnp.dot(g_cur, w2, preferred_element_type=F32)
                acc = p if acc is None else p + acc
            else:
                b2 = jnp.broadcast_to(b2_s[...].astype(F32).reshape(1, D), (8, D))
                for r in range(nsb):
                    rr = pl.multiple_of(r0 + r * SB3, SB3)
                    b2r = _tie(b2, next_ln())
                    p = jnp.dot(g_cur[r * SB3:(r + 1) * SB3], w2, preferred_element_type=F32)
                    res = p + acc[r * SB3:(r + 1) * SB3] + h_s[pl.ds(rr, SB3), :]
                    res = (res.reshape(SB3 // 8, 8, D) + b2r[None]).reshape(SB3, D)
                    x_s[pl.ds(rr, SB3), :] = res.astype(BF)
                    o_copy(rr).start()
        while blocks:
            next_ln()
        return carry

    lax.fori_loop(0, n3, mlp_body, 0)
    for r in range(S // SB3):
        o_copy(r * SB3).wait()


@jax.jit
def pallas_sequential_preLN__softmax_full_mha__mixer_channel_mlp__prompt_kernel(
    A_x: jax.Array,
    A_wqkv: jax.Array,
    A_wo: jax.Array,
    B_x: jax.Array,
    B_w1: jax.Array,
    B_b1: jax.Array,
    B_w2: jax.Array,
    B_b2: jax.Array,
):
    B, S, D = A_x.shape
    F = B_w1.shape[1]
    assert B == 1 and D % 128 == 0 and (D // H) * HPG == 128
    DH = D // H
    G = D // 128
    any_spec = pl.BlockSpec(memory_space=pl.ANY)
    return pl.pallas_call(
        functools.partial(_kernel, S=S, D=D, F=F),
        out_shape=jax.ShapeDtypeStruct((B, S, D), A_x.dtype),
        in_specs=[any_spec] * 7,
        out_specs=any_spec,
        scratch_shapes=[
            pltpu.VMEM((NS, S, TQ), F32),
            pltpu.VMEM((G, S, 128), BF),
            pltpu.VMEM((H, DH, S), BF),
            pltpu.VMEM((H, DH, S), BF),
            pltpu.VMEM((G, S, 128), BF),
            pltpu.VMEM((S, D), F32),
            pltpu.VMEM((TM3, D), BF),
            pltpu.VMEM((TM3, D), BF),
            pltpu.VMEM((S, D), BF),
            pltpu.VMEM((2, TM1, D), BF),
            pltpu.VMEM((D, 3 * D), BF),
            pltpu.VMEM((D, D), BF),
            pltpu.VMEM((D, F), BF),
            pltpu.VMEM((F, D), BF),
            pltpu.VMEM((NS * DH, TQ), F32),
            pltpu.VMEM((NS, 1, TQ), F32),
            pltpu.VMEM((F,), BF),
            pltpu.VMEM((D,), BF),
            pltpu.SemaphoreType.DMA((TM1 // SB1 + S // TM1 - 1,)),
            pltpu.SemaphoreType.DMA((3 * D // TN1 + 1,)),
            pltpu.SemaphoreType.DMA((5,)),
            pltpu.SemaphoreType.DMA(()),
        ],
        compiler_params=pltpu.CompilerParams(vmem_limit_bytes=120 * 1024 * 1024),
    )(A_x, A_wqkv, A_wo, B_w1, B_b1, B_w2, B_b2)
```

```python
import functools

import jax
import jax.numpy as jnp
from jax import lax
import jax.experimental.pallas as pl
import jax.experimental.pallas.tpu as pltpu

BF = jnp.bfloat16
F32 = jnp.float32

H = 32
EPS = 1e-5
LOG2E = 1.4426950408889634

TM1 = 512
TN1 = 512
SB1 = 128
LNB = 32
TQ = 512
CK = 128
HPG = 4
NS = 8
OPM = 128
OPN = 256
TM3 = 256
FC = 512
SB3 = 128


def _layernorm(x):
    mu = jnp.mean(x, axis=-1, keepdims=True)
    xc = x - mu
    var = jnp.mean(xc * xc, axis=-1, keepdims=True)
    return xc * lax.rsqrt(var + EPS)


def _gelu_tanh(x):
    c = 0.7978845608028654
    return 0.5 * x * (1.0 + jnp.tanh(c * (x + 0.044715 * (x * x * x))))


def _tie(v, y):
    if y is None:
        return v
    w = v.shape[1]
    t = jnp.max(y.reshape(y.shape[0] // 8, 8, y.shape[1]), axis=0)
    tw = t[:, :w]
    for k in range(1, y.shape[1] // w):
        tw = jnp.maximum(tw, t[:, k * w:(k + 1) * w])
    return jnp.where(tw > jnp.inf, tw, v)


def _interleave(main, extra):
    n, k = len(main), len(extra)
    done = 0
    for idx, fn in enumerate(main):
        fn()
        want = ((idx + 1) * k) // n
        while done < want:
            extra[done]()
            done += 1


def _kernel(x_hbm, wqkv_hbm, wo_hbm, w1_hbm, b1_hbm, w2_hbm, b2_hbm, out_hbm,
            s_buf, k_s, qt_s, vt_s, o_s, h_s, y_s, yn_s, x_s, xn_s, wqkv_s, wo_s, w1_s, w2_s,
            ot_t, m_s, b1_s, b2_s,
            sem_x, sem_w, sem_p, sem_o, *, S, D, F):
    DH = D // H
    G = D // 128
    qscale = (DH ** -0.5) * LOG2E
    n1 = S // TM1
    npart = D // TN1
    w_order = ([npart + n for n in range(npart)] + list(range(npart))
               + [2 * npart + n for n in range(npart)])

    nsb1 = TM1 // SB1
    x_rows = ([(r * SB1, SB1) for r in range(nsb1)]
              + [(i * TM1, TM1) for i in range(1, n1)])
    c_first = w_order[0] * TN1
    wsb = TN1 // 2
    dma_order = [w_order[2], w_order[1]] + w_order[3:]
    w_cols = ([(c_first + b * wsb, wsb) for b in range(2)]
              + [(n * TN1, TN1) for n in dma_order])

    def x_copy(i):
        r0, nr = x_rows[i]
        return pltpu.make_async_copy(x_hbm.at[0, pl.ds(r0, nr), :],
                                     x_s.at[pl.ds(r0, nr), :], sem_x.at[i])

    def w_copy(n):
        c0, nc = w_cols[n]
        return pltpu.make_async_copy(wqkv_hbm.at[:, pl.ds(c0, nc)],
                                     wqkv_s.at[:, pl.ds(c0, nc)], sem_w.at[n])

    p_copies = [pltpu.make_async_copy(src, dst, sem_p.at[n]) for n, (src, dst) in enumerate(
        ((wo_hbm, wo_s), (w1_hbm, w1_s), (w2_hbm, w2_s), (b1_hbm, b1_s), (b2_hbm, b2_s)))]

    def o_copy(r):
        return pltpu.make_async_copy(x_s.at[pl.ds(r, SB3), :],
                                     out_hbm.at[0, pl.ds(r, SB3), :], sem_o)

    def ln1(i, r):
        for rr in range(r * SB1, (r + 1) * SB1, LNB):
            xb = x_s[i * TM1 + rr:i * TM1 + rr + LNB, :].astype(F32)
            xn_s[i % 2, rr:rr + LNB, :] = _layernorm(xb).astype(BF)

    def proj(i, n, r=None, cols=None):
        c0, nc = n * TN1, TN1
        if cols is not None:
            c0, nc = c0 + cols[0] * wsb, (cols[1] - cols[0]) * wsb
        part = c0 // D
        lo, hi = (0, TM1) if r is None else (r[0] * SB1, r[1] * SB1)
        rows = slice(i * TM1 + lo, i * TM1 + hi)
        xn = xn_s[i % 2, lo:hi, :]
        if part == 1:
            kb = jnp.dot(xn, wqkv_s[:, c0:c0 + nc], preferred_element_type=F32).astype(BF)
            for g in range(nc // 128):
                k_s[(c0 - D) // 128 + g, rows, :] = kb[:, g * 128:(g + 1) * 128]
        else:
            t = lax.dot_general(wqkv_s[:, c0:c0 + nc], xn,
                                (((0,), (1,)), ((), ())), preferred_element_type=F32)
            if part == 0:
                t = t * qscale
            t = t.astype(BF)
            dst = qt_s if part == 0 else vt_s
            for hh in range(nc // DH):
                dst[(c0 - part * D) // DH + hh, :, rows] = t[hh * DH:(hh + 1) * DH, :]

    def head_work(i):
        def blk(r):
            def fn():
                ln1(i, r)
                proj(i, w_order[0], (r, r + 1))
            return fn
        return [blk(r) for r in range(nsb1)]

    def tail_work(i, first=1):
        return [functools.partial(proj, i, n) for n in w_order[first:]]

    hb = nsb1 // 2
    for r in range(hb):
        x_copy(r).start()
    for r in range(hb):
        x_copy(r).wait()
        if r == 0:
            w_copy(0).start()
        if r == hb - 1:
            for rr in range(hb, nsb1):
                x_copy(rr).start()
        ln1(0, r)
    w_copy(0).wait()
    for n in range(1, len(w_cols)):
        w_copy(n).start()
    proj(0, w_order[0], (0, hb), (0, 1))
    for r in range(hb, nsb1):
        x_copy(r).wait()
    for r in range(nsb1, len(x_rows)):
        x_copy(r).start()
    for r in range(hb, nsb1):
        ln1(0, r)
        proj(0, w_order[0], (r, r + 1), (0, 1))
    w_copy(1).wait()
    for c in p_copies:
        c.start()
    proj(0, w_order[0], None, (1, 2))
    w_copy(2).wait()
    proj(0, w_order[2])
    w_copy(3).wait()
    w_copy(4).wait()
    proj(0, w_order[1], (0, hb))
    proj(0, w_order[3])
    for n in range(5, len(w_cols)):
        w_copy(n).wait()
    x_copy(nsb1).wait()
    proj(0, w_order[1], (hb, nsb1))
    _interleave(tail_work(0, 4), head_work(1))
    for r in range(nsb1 + 1, len(x_rows)):
        x_copy(r).wait()
    for i in range(1, n1):
        _interleave(tail_work(i), head_work(i + 1) if i + 1 < n1 else [])

    nq = S // TQ
    nck = S // CK
    gpb = NS // HPG
    gb = G // gpb
    nb = nq * gb

    def load_qm(h, j, qi):
        qh = qt_s[h, :, pl.ds(pl.multiple_of(qi * TQ, TQ), TQ)]
        parts = []
        if j > 0:
            parts.append(jnp.zeros((DH * j, TQ), BF))
        parts.append(qh)
        if j < HPG - 1:
            parts.append(jnp.zeros((DH * (HPG - 1 - j), TQ), BF))
        return jnp.concatenate(parts, axis=0)

    def qk_chunk(i, g, qm, c, mrun):
        s = jnp.dot(k_s[g, c * CK:(c + 1) * CK, :], qm, preferred_element_type=F32)
        s_buf[i, c * CK:(c + 1) * CK, :] = s
        cm = jnp.max(s.reshape(CK // 8, 8, TQ), axis=0)
        return cm if mrun is None else jnp.maximum(mrun, cm)

    def p_chunk(i, c, m, lrun):
        ps = [None] * (CK // 16)
        cl = None
        for r in reversed(range(CK // 16)):
            s = s_buf[i, c * CK + r * 16:c * CK + (r + 1) * 16, :]
            p = jnp.exp2(s - m)
            cl = p[8:16] if cl is None else cl + p[8:16]
            cl = cl + p[0:8]
            ps[r] = p
        lrun = cl if lrun is None else lrun + cl
        return lrun, jnp.concatenate(ps, axis=0).astype(BF)

    def pv_chunk(h, c, pb, acc):
        o = jnp.dot(vt_s[h, :, c * CK:(c + 1) * CK], pb, preferred_element_type=F32)
        return o if acc is None else o + acc

    def flush_o(u):
        qi, g0 = u // gb, (u % gb) * gpb
        for gg in range(gpb):
            o_s[g0 + gg, pl.ds(pl.multiple_of(qi * TQ, TQ), TQ), :] = (
                ot_t[gg * 128:(gg + 1) * 128, :].T.astype(BF))

    def attn_work(u, do_pv, do_qk):
        if do_pv:
            qi, g0 = u // gb, (u % gb) * gpb
        if do_qk:
            qin, gn0 = (u + 1) // gb, ((u + 1) % gb) * gpb
        work = []
        for i in range(NS):
            j = i % HPG
            st = {}

            def step(c, i=i, j=j, st=st):
                if do_pv:
                    h = (g0 + i // HPG) * HPG + j
                    if c == 0:
                        st['m'] = m_s[i]
                        st['l'] = st['acc'] = None
                    st['l'], pb = p_chunk(i, c, st['m'], st['l'])
                if do_qk:
                    gn = gn0 + i // HPG
                    if c == 0:
                        st['qm'] = load_qm(gn * HPG + j, j, qin)
                        st['mrun'] = None
                    st['mrun'] = qk_chunk(i, gn, st['qm'], c, st['mrun'])
                if do_pv:
                    st['acc'] = pv_chunk(h, c, pb, st['acc'])
                if c == nck - 1:
                    if do_pv:
                        l = jnp.sum(st['l'], axis=0, keepdims=True)
                        ot_t[i * DH:(i + 1) * DH, :] = st['acc'] / l
                    if do_qk:
                        m_s[i] = jnp.max(st['mrun'], axis=0, keepdims=True)
            work += [functools.partial(step, c) for c in range(nck)]
        return work

    ot_t[...] = jnp.zeros(ot_t.shape, F32)
    for fn in attn_work(-1, False, True):
        fn()

    def attn_loop(u, carry):
        flush_o(jnp.maximum(u - 1, 0))
        for fn in attn_work(u, True, True):
            fn()
        return carry

    lax.fori_loop(0, nb - 1, attn_loop, 0)

    def op_work(r0, nrows, ncols):
        rows = slice(r0, r0 + nrows)

        def piece(n):
            def fn():
                o = jnp.concatenate([o_s[g, rows, :] for g in range(G)], axis=1)
                cols = slice(n * ncols, (n + 1) * ncols)
                at = jnp.dot(o, wo_s[:, cols], preferred_element_type=F32)
                h_s[rows, cols] = x_s[rows, cols].astype(F32) + at
            return fn
        return [piece(n) for n in range(D // ncols)]

    def op_small_work(r0):
        rows = slice(r0, r0 + CK)

        def piece(n, g):
            def fn():
                cols = slice(n * TQ, (n + 1) * TQ)
                at = jnp.dot(o_s[g, rows, :], wo_s[g * 128:(g + 1) * 128, cols],
                             preferred_element_type=F32)
                prev = x_s[rows, cols].astype(F32) if g == 0 else h_s[rows, cols]
                h_s[rows, cols] = prev + at
            return fn
        return [piece(n, g) for n in range(D // TQ) for g in range(G)]

    def ln2(r0, b):
        hb = h_s[pl.ds(pl.multiple_of(r0 + b * LNB, LNB), LNB), :]
        y = _layernorm(_layernorm(hb))
        yn_s[b * LNB:(b + 1) * LNB, :] = y.astype(BF)
        return y

    for c in p_copies:
        c.wait()
    flush_o(nb - 2)
    epi = attn_work(nb - 1, True, False)
    fused_rows = (len(epi) // (G * (D // TQ))) * CK
    extra = []
    for r0 in range(0, fused_rows, CK):
        extra += op_small_work(r0)
    _interleave(extra, epi)
    flush_o(nb - 1)
    rest = []
    for r0 in range(fused_rows, S, OPM):
        rest += op_work(r0, OPM, OPN)
    nln = TM3 // LNB
    _interleave(rest, [functools.partial(ln2, 0, b) for b in range(nln)])

    n3 = S // TM3
    nf = F // FC
    nsb = TM3 // SB3

    def mlp_body(i, carry):
        r0 = pl.multiple_of(i * TM3, TM3)
        rn = jnp.minimum(i + 1, n3 - 1) * TM3
        y_s[...] = yn_s[...]

        blocks = list(range(nln))

        def next_ln():
            return ln2(rn, blocks.pop(0)) if blocks else None

        def up(c, dep):
            b = b1_s[pl.ds(c * FC, FC)].astype(F32).reshape(1, FC)
            b = _tie(jnp.broadcast_to(b, (8, FC)), dep)
            a = jnp.dot(y_s[...], w1_s[:, c * FC:(c + 1) * FC],
                        preferred_element_type=F32)
            a = (a.reshape(TM3 // 8, 8, FC) + b[None]).reshape(TM3, FC)
            return _gelu_tanh(a).astype(BF)

        acc = None
        g_next = up(0, None)
        for c in range(nf):
            g_cur = g_next
            if c + 1 < nf:
                g_next = up(c + 1, next_ln())
            w2 = w2_s[c * FC:(c + 1) * FC, :]
            if c + 1 < nf:
                p = jnp.dot(g_cur, w2, preferred_element_type=F32)
                acc = p if acc is None else p + acc
            else:
                b2 = jnp.broadcast_to(b2_s[...].astype(F32).reshape(1, D), (8, D))
                for r in range(nsb):
                    rr = pl.multiple_of(r0 + r * SB3, SB3)
                    b2r = _tie(b2, next_ln())
                    p = jnp.dot(g_cur[r * SB3:(r + 1) * SB3], w2, preferred_element_type=F32)
                    res = p + acc[r * SB3:(r + 1) * SB3] + h_s[pl.ds(rr, SB3), :]
                    res = (res.reshape(SB3 // 8, 8, D) + b2r[None]).reshape(SB3, D)
                    x_s[pl.ds(rr, SB3), :] = res.astype(BF)
                    o_copy(rr).start()
        while blocks:
            next_ln()
        return carry

    lax.fori_loop(0, n3, mlp_body, 0)
    for r in range(S // SB3):
        o_copy(r * SB3).wait()


@jax.jit
def pallas_sequential_preLN__softmax_full_mha__mixer_channel_mlp__prompt_kernel(
    A_x: jax.Array,
    A_wqkv: jax.Array,
    A_wo: jax.Array,
    B_x: jax.Array,
    B_w1: jax.Array,
    B_b1: jax.Array,
    B_w2: jax.Array,
    B_b2: jax.Array,
):
    B, S, D = A_x.shape
    F = B_w1.shape[1]
    assert B == 1 and D % 128 == 0 and (D // H) * HPG == 128
    DH = D // H
    G = D // 128
    any_spec = pl.BlockSpec(memory_space=pl.ANY)
    return pl.pallas_call(
        functools.partial(_kernel, S=S, D=D, F=F),
        out_shape=jax.ShapeDtypeStruct((B, S, D), A_x.dtype),
        in_specs=[any_spec] * 7,
        out_specs=any_spec,
        scratch_shapes=[
            pltpu.VMEM((NS, S, TQ), F32),
            pltpu.VMEM((G, S, 128), BF),
            pltpu.VMEM((H, DH, S), BF),
            pltpu.VMEM((H, DH, S), BF),
            pltpu.VMEM((G, S, 128), BF),
            pltpu.VMEM((S, D), F32),
            pltpu.VMEM((TM3, D), BF),
            pltpu.VMEM((TM3, D), BF),
            pltpu.VMEM((S, D), BF),
            pltpu.VMEM((2, TM1, D), BF),
            pltpu.VMEM((D, 3 * D), BF),
            pltpu.VMEM((D, D), BF),
            pltpu.VMEM((D, F), BF),
            pltpu.VMEM((F, D), BF),
            pltpu.VMEM((NS * DH, TQ), F32),
            pltpu.VMEM((NS, 1, TQ), F32),
            pltpu.VMEM((F,), BF),
            pltpu.VMEM((D,), BF),
            pltpu.SemaphoreType.DMA((TM1 // SB1 + S // TM1 - 1,)),
            pltpu.SemaphoreType.DMA((3 * D // TN1 + 1,)),
            pltpu.SemaphoreType.DMA((5,)),
            pltpu.SemaphoreType.DMA(()),
        ],
        compiler_params=pltpu.CompilerParams(vmem_limit_bytes=120 * 1024 * 1024),
    )(A_x, A_wqkv, A_wo, B_w1, B_b1, B_w2, B_b2)
```
